```python
import os as _os
_os.environ.setdefault("JAX_PLATFORMS", "cpu")
import jax
import jax.numpy as jnp

def _softmax(x, axis=-1):
    return jax.nn.softmax(x, axis=axis)
def _gelu(x):
    return jax.nn.gelu(x, approximate=True)
def _silu(x):
    return jax.nn.silu(x)
def _sigmoid(x):
    return jax.nn.sigmoid(x)
def _layernorm(x, axis=-1, eps=1e-5):
    m = jnp.mean(x, axis=axis, keepdims=True)
    v = jnp.var(x, axis=axis, keepdims=True)
    return (x - m) / jnp.sqrt(v + eps)
def _scatter_add(tgt, idx, src, axis=0):
    return tgt.at[idx].add(src)
def _segment_sum(src, seg, n):
    return jax.ops.segment_sum(src, seg, n)
class _Rng:
    def __init__(self, key):
        self._k = key
    def _next(self):
        self._k, sub = jax.random.split(self._k)
        return sub
    def normal(self, shape):
        return jax.random.normal(self._next(), shape, dtype=jnp.bfloat16)
    def randint(self, lo, hi, shape):
        return jax.random.randint(self._next(), shape, lo, hi, dtype=jnp.int32)
    def uniform(self, shape, lo=0.0, hi=1.0):
        return jax.random.uniform(self._next(), shape, jnp.bfloat16, lo, hi)
    def permutation(self, n):
        return jax.random.permutation(self._next(), n)


kernel_name = 'sequential_preLN__mha_block__dense_activation_squared_relu__prompt'

def setup_inputs():
    _rng = _Rng(jax.random.key(int.from_bytes(__import__("os").urandom(4), "little")))
    _w = (lambda a: (lambda t: t.astype(jnp.bfloat16) if jnp.issubdtype(t.dtype, jnp.floating) else t)(jnp.asarray(a)))
    def _A_setup():
        B, S, D, H = 1, 2048, 448, 16
        return {
            "x": _w((lambda *s: _rng.normal(s) * 0.05)(B, S, D)),
            "wqkv": _w((lambda *s: _rng.normal(s) * 0.05)(D, 3 * D)),
            "wo": _w((lambda *s: _rng.normal(s) * 0.05)(D, D)),
        }
    _A_in = _A_setup()

    def _B_setup():
        B, S, D, F = 1, 2048, 448, 1792
        return {
            "x": _w((lambda *s: _rng.normal(s) * 0.05)(B, S, D)),
            "w1": _w((lambda *s: _rng.normal(s) * 0.05)(D, F)),
            "b1": _w((lambda *s: _rng.normal(s) * 0.05)(F)),
            "w2": _w((lambda *s: _rng.normal(s) * 0.05)(F, D)),
            "b2": _w((lambda *s: _rng.normal(s) * 0.05)(D)),
        }
    _B_in = _B_setup()

    return {
        "A_x": _A_in["x"],
        "A_wqkv": _A_in["wqkv"],
        "A_wo": _A_in["wo"],
        "B_x": _B_in["x"],
        "B_w1": _B_in["w1"],
        "B_b1": _B_in["b1"],
        "B_w2": _B_in["w2"],
        "B_b2": _B_in["b2"],
    }

def reference(A_x, A_wqkv, A_wo, B_x, B_w1, B_b1, B_w2, B_b2):
    def _A_ref(x, wqkv, wo):
        B, S, D = x.shape
        H = 16
        Dh = D // H
        qkv = (lambda x, *d: x.transpose(*d))((x @ wqkv).reshape(B, S, 3, H, Dh), 2, 0, 3, 1, 4)
        q, k, v = qkv[0], qkv[1], qkv[2]
        scores = jnp.einsum("bhqd,bhkd->bhqk", q, k) * (Dh ** -0.5)
        p = _softmax(scores, axis=-1)
        o = jnp.einsum("bhqk,bhkd->bhqd", p, v)
        return (lambda x, *d: x.transpose(*d))(o, 0, 2, 1, 3).reshape(B, S, D) @ wo

    def _B_ref(x, w1, b1, w2, b2):
        h = jnp.einsum("bsd,df->bsf", x, w1) + b1
        zero = jnp.zeros_like(h)
        r = jnp.where(h > zero, h, zero)
        h = r * r
        out = jnp.einsum("bsf,fd->bsd", h, w2) + b2
        return out

    x = A_x
    h = x + _A_ref(_layernorm(x, axis=-1), A_wqkv, A_wo)
    h2 = h + _B_ref(_layernorm(h, axis=-1), B_w1, B_b1, B_w2, B_b2)
    return h2
```

```python
import jax
import jax.numpy as jnp
from jax import lax
import jax.experimental.pallas as pl
import jax.experimental.pallas.tpu as pltpu

S, D, H, DH, F = 2048, 448, 16, 28, 1792
EPS = 1e-5
LOG2E = 1.4426950408889634
bf16, f32, u32 = jnp.bfloat16, jnp.float32, jnp.uint32

HP = 32
DP = H * HP
G = 4
GW = 4 * DH
TQ = 512
NQ = S // TQ
NT = TQ // 128
KC = 128
NKC = S // KC
HPI = 8
NIT = H // HPI
GPI = HPI // 4
DIST = 8

VK = 16
OCH = (4, 5, 6, 7, 9, 10, 11, 12, 13, 14, 15)
NE = 6
NOC = len(OCH)
_REST = [c for c in range(NKC) if c not in OCH]
CORD = _REST[:3] + list(OCH[NE:]) + list(OCH[:NE]) + _REST[3:]
EHEADS = [(hh, u) for hh in range(NIT) for u in range(1, HPI)]

XSPLIT = ((0, 256), (256, 512), (512, 1024), (1024, 1536), (1536, 2048))
WSPLIT = ((0, 512), (512, 896), (896, 1344))


def _pk(x):
    return pltpu.bitcast(x, u32)


def _up(x):
    return pltpu.bitcast(x, bf16)


def _dot(a, b):
    return jnp.dot(a, b, preferred_element_type=f32)


def _ln(x):
    m = jnp.sum(x, axis=0, keepdims=True) * (1.0 / D)
    xc = x - m
    v = jnp.sum(xc * xc, axis=0, keepdims=True) * (1.0 / D)
    return xc * lax.rsqrt(v + EPS)


def _pad_head_rows(w, fill):
    parts = []
    for h in range(H):
        parts += [w[DH * h:DH * (h + 1), :], fill]
    return jnp.concatenate(parts, axis=0)


def _first_row(row, rows):
    r = lax.broadcasted_iota(jnp.int32, (rows, row.shape[1]), 0)
    return jnp.where(r == 0, row, 0.0)


def _kernel(xT_hbm, wqkv_hbm, wo_hbm, w1_hbm, b1_hbm, w2T_hbm, b2_hbm,
            o_hbm,
            k_sc, qT_sc, vT_sc, oT_sc, spre_sc, sve_sc, sva_sc, qf_sc, kb_sc, y_sc,
            xT_ref, wqkv_ref, wo_ref, w1_ref, w2T_ref, wqkvT_sc, woT_sc, w1T_sc, b2_sc, kt_sc,
            b1_ref, b2_ref, sems, osem):
    i = pl.program_id(0)
    rowq = lax.broadcasted_iota(jnp.int32, (64, TQ), 0)

    def masked_q(blk, g, j):
        qg = qT_sc[blk, g]
        keep = (rowq >= (DH // 2) * j) & (rowq < (DH // 2) * (j + 1))
        return _up(jnp.where(keep, qg, jnp.zeros_like(qg)))

    def qk(g, k0, k1, qm):
        return _dot(_up(k_sc[g, k0 // 2:k1 // 2, :]), qm)

    def vpu_scores(blk, hlist, o0, o1, rows):
        prev = jnp.zeros((rows, 128), f32)
        for hh, u in hlist:
            for t in range(NT):
                for v0 in range(o0 * VK, o1 * VK, rows):
                    a = prev * 0.0
                    for d in range(DH):
                        r = u * DH + d
                        a = a + kb_sc[hh, u, d, v0:v0 + rows, :] * qf_sc[blk, hh, r:r + 1, t * 128:(t + 1) * 128]
                    if o0 >= NE:
                        sva_sc[u, v0 - NE * VK:v0 - NE * VK + rows, t * 128:(t + 1) * 128] = a
                    else:
                        sve_sc[hh, u - 1, v0:v0 + rows, t * 128:(t + 1) * 128] = a
                    prev = a

    @pl.when(i == 0)
    def _prologue():
        def cp_x(n, sem):
            a, b = XSPLIT[n]
            return pltpu.make_async_copy(xT_hbm.at[:, a:b], xT_ref.at[:, a:b], sems.at[sem])

        def cp_w(n, sem):
            a, b = WSPLIT[n]
            return pltpu.make_async_copy(wqkv_hbm.at[:, a:b], wqkv_ref.at[:, a:b], sems.at[sem])

        def cp(src, dst, sem):
            return pltpu.make_async_copy(src, dst, sems.at[sem])

        stages = [
            [cp_x(0, 0)],
            [cp_w(0, 1)],
            [cp_x(1, 2), cp_w(1, 2)],
            [cp_w(2, 3), cp_x(2, 3)],
            [cp_x(3, 4), cp_x(4, 4), cp(wo_hbm, wo_ref, 4), cp(b2_hbm, b2_ref, 4), cp(b1_hbm, b1_ref, 4),
             cp(w1_hbm, w1_ref, 4)],
            [cp(w2T_hbm, w2T_ref, 5)],
        ]
        for st in stages:
            for c in st:
                c.start()

        def wait(n):
            for c in stages[n]:
                c.wait()

        def ln1(n):
            a, b = XSPLIT[n]
            return _ln(xT_ref[:, a:b].astype(f32)).astype(bf16)

        def transpose_w(n):
            a, b = WSPLIT[n]
            wqkvT_sc[a // 2:b // 2, :] = _pk(wqkv_ref[:, a:b].T)

        def proj(r0, r1, xn):
            return _dot(_up(wqkvT_sc[r0 // 2:r1 // 2, :]), xn)

        def proj_q(n, xn, g0=0, g1=G):
            a, b = XSPLIT[n]
            cols = slice(a % TQ, a % TQ + b - a)
            zpad = jnp.zeros((128 - GW, b - a), f32)
            qT = proj(GW * g0, GW * g1, xn) * (DH ** -0.5 * LOG2E)
            for g in range(g0, g1):
                qg = qT[GW * (g - g0):GW * (g - g0 + 1), :]
                qf_sc[a // TQ, g // GPI, GW * (g % GPI):GW * (g % GPI + 1), cols] = qg
                qT_sc[a // TQ, g, :, cols] = _pk(jnp.concatenate([qg, zpad], axis=0).astype(bf16))

        def proj_k(n, xn):
            a, b = XSPLIT[n]
            zpad = jnp.zeros((128 - GW, b - a), f32)
            kT = proj(D, 2 * D, xn)
            for g in range(G):
                kg = jnp.concatenate([kT[GW * g:GW * (g + 1), :], zpad], axis=0).astype(bf16)
                k_sc[g, a // 2:b // 2, :] = _pk(kg.T)

        def proj_v(n, xn):
            a, b = XSPLIT[n]
            ones = _first_row(jnp.ones((1, b - a), f32), HP - DH)
            vT_sc[:, a:b] = _pk(_pad_head_rows(proj(2 * D, 3 * D, xn), ones).astype(bf16))

        def vkeys(g, o0, o1):
            return jnp.concatenate(
                [k_sc[g, ((OCH[o] + 1) * KC - VK) // 2:(OCH[o] + 1) * KC // 2, :] for o in range(o0, o1)], axis=0)

        def broadcast_k(o0, o1, via_transpose):
            for j in range(4):
                sel = [(g, o0 if (4 * g + j) % HPI else max(o0, NE)) for g in range(G)]
                sel = [(g, lo) for g, lo in sel if lo < o1]
                ksel = jnp.concatenate([vkeys(g, lo, o1) for g, lo in sel], axis=0)
                nk = 2 * ksel.shape[0]
                if via_transpose:
                    kt_sc[:, 0:nk] = _up(ksel).T.astype(f32)
                for d in range(DH):
                    lane = DH * j + d
                    if via_transpose:
                        kb = jnp.broadcast_to(kt_sc[lane:lane + 1, 0:nk], (128, nk)).astype(bf16).T.astype(f32)
                    else:
                        kb = _up(jnp.broadcast_to(ksel[:, lane:lane + 1], ksel.shape)).astype(f32)
                    r0 = 0
                    for g, lo in sel:
                        h = 4 * g + j
                        kb_sc[h // HPI, h % HPI, d, lo * VK:o1 * VK, :] = kb[r0:r0 + (o1 - lo) * VK, :]
                        r0 += (o1 - lo) * VK

        def first_scores(hlist, o0, o1):
            for hh, u in hlist:
                h = hh * HPI + u
                s = _dot(_up(vkeys(h // 4, o0, o1)), masked_q(0, h // 4, h % 4))
                if o0 >= NE:
                    sva_sc[u, (o0 - NE) * VK:(o1 - NE) * VK, :] = s
                else:
                    sve_sc[hh, u - 1, o0 * VK:o1 * VK, :] = s

        wait(0)
        xn0 = ln1(0)
        wait(1)
        transpose_w(0)
        proj_q(0, xn0, 0, 3)
        wait(2)
        proj_q(0, xn0, 3, 4)
        transpose_w(1)
        xn1 = ln1(1)
        proj_k(0, xn0)
        proj_q(1, xn1)
        wait(3)
        proj_k(1, xn1)
        transpose_w(2)
        xn2 = ln1(2)
        proj_k(2, xn2)
        broadcast_k(0, 4, True)
        proj_v(0, xn0)
        proj_v(1, xn1)
        proj_q(2, xn2)
        proj_v(2, xn2)
        wait(4)
        woT_sc[...] = _pk(_pad_head_rows(wo_ref[...].astype(f32), jnp.zeros((HP - DH, D), f32)).astype(bf16).T)
        b2_sc[...] = jnp.broadcast_to(b2_ref[...].astype(f32).reshape(1, D), (128, D)).T
        b1_rows = _first_row(b1_ref[...].astype(f32).reshape(1, F), DP - D).astype(bf16)
        w1T_sc[...] = _pk(jnp.concatenate([w1_ref[...], b1_rows], axis=0).T)
        xn3 = ln1(3)
        first_scores(EHEADS, 0, 4)
        proj_k(3, xn3)
        xn4 = ln1(4)
        proj_k(4, xn4)
        broadcast_k(4, 7, False)
        broadcast_k(7, NOC, True)
        proj_v(3, xn3)
        proj_q(3, xn3)
        proj_v(4, xn4)
        proj_q(4, xn4)
        first_scores(EHEADS, 4, NE)
        first_scores([(0, u) for u in range(HPI)], NE, NOC)
        qm = masked_q(0, 0, 0)
        for w in range(DIST):
            c = CORD[w // NT]
            spre_sc[w] = qk(0, c * KC, (c + 1) * KC, qm[:, (w % NT) * 128:(w % NT + 1) * 128])
        wait(5)

    def attention(hh, carry):
        work = [(u, c, t) for u in range(HPI) for c in CORD for t in range(NT)]
        n = len(work)
        per_head = NKC * NT
        nxt = i * NIT + hh + 1
        nblk = jnp.minimum(nxt // NIT, NQ - 1)
        nhh = nxt % NIT
        qms = {}

        def scores(w):
            u, c, t = work[w % n]
            cols = slice(t * 128, (t + 1) * 128)
            if w >= n:
                if "next" not in qms:
                    qms["next"] = masked_q(nblk, nhh * GPI, 0)
                return qk(nhh * GPI, c * KC, (c + 1) * KC, qms["next"][:, cols])
            g = hh * GPI + u // 4
            if u not in qms:
                qms[u] = masked_q(i, g, u % 4)
            qm = qms[u][:, cols]
            if c in (OCH if u else OCH[NE:]):
                o = OCH.index(c)
                if o < NE:
                    sv = sve_sc[hh, u - 1, o * VK:(o + 1) * VK, cols]
                else:
                    sv = sva_sc[u, (o - NE) * VK:(o - NE + 1) * VK, cols]
                return jnp.concatenate([qk(g, c * KC, (c + 1) * KC - VK, qm), sv], axis=0)
            return qk(g, c * KC, (c + 1) * KC, qm)

        svals = {w: spre_sc[w] for w in range(DIST)}
        state = {}
        for w, (u, c, t) in enumerate(work):
            s = svals.pop(w)
            m, acc = state.get((u, t), (None, None))
            cm = jnp.max(s, axis=0, keepdims=True)
            m_new = cm if m is None else jnp.maximum(m, cm)
            p = jnp.exp2(s - m_new).astype(bf16)
            if w + DIST < n:
                svals[w + DIST] = scores(w + DIST)
            else:
                spre_sc[w + DIST - n] = scores(w + DIST)
            h0 = pl.multiple_of((hh * HPI + u) * (HP // 2), HP // 2)
            pv = _dot(_up(vT_sc[pl.ds(h0, HP // 2), c * KC:(c + 1) * KC]), p)
            acc = pv if m is None else acc * jnp.exp2(m - m_new) + pv
            state[(u, t)] = (m_new, acc)
            if w % per_head >= per_head - NT:
                l = acc[DH:DH + 1, :]
                r = pl.reciprocal(l, approx=True)
                r = r * (2.0 - l * r)
                oT_sc[pl.ds(h0, HP // 2), t * 128:(t + 1) * 128] = _pk((acc * r).astype(bf16))
        vpu_scores(nblk, [(nhh, u) for u in range(HPI)], NE, NOC, 8)
        return carry

    lax.fori_loop(0, NIT, attention, 0)

    q0 = pl.multiple_of(i * TQ, TQ)
    hT = xT_ref[:, pl.ds(q0, TQ)].astype(f32) + _dot(_up(woT_sc[...]), _up(oT_sc[...]))
    ones = _first_row(jnp.ones((1, 128), f32), DP - D)
    for t in range(NT):
        ht = hT[:, t * 128:(t + 1) * 128]
        hn = jnp.concatenate([_ln(ht), ones], axis=0).astype(bf16)
        u = jnp.maximum(_dot(_up(w1T_sc[...]), hn), 0.0)
        y = ht + b2_sc[...] + _dot(w2T_ref[...], (u * u).astype(bf16))
        y_sc[:, pl.ds(pl.multiple_of(q0 + t * 128, 128), 128)] = y.astype(bf16)
        if t >= NT - 2:
            c0, cw = (0, (NT - 1) * 128) if t == NT - 2 else (t * 128, 128)
            cols = pl.ds(pl.multiple_of(q0 + c0, 128), cw)
            pltpu.make_async_copy(y_sc.at[:, cols], o_hbm.at[:, cols], osem.at[0]).start()
    vpu_scores(jnp.minimum(i + 1, NQ - 1), EHEADS, 0, NE, 24)

    @pl.when(i == NQ - 1)
    def _():
        pltpu.make_async_copy(y_sc, o_hbm, osem.at[0]).wait()


@jax.jit
def pallas_sequential_preLN__mha_block__dense_activation_squared_relu__prompt_kernel(
    A_x: jax.Array,
    A_wqkv: jax.Array,
    A_wo: jax.Array,
    B_x: jax.Array,
    B_w1: jax.Array,
    B_b1: jax.Array,
    B_w2: jax.Array,
    B_b2: jax.Array,
):
    del B_x
    hbm = pl.BlockSpec(memory_space=pl.ANY)
    outT = pl.pallas_call(
        _kernel,
        grid=(NQ,),
        in_specs=[hbm] * 7,
        out_specs=hbm,
        out_shape=jax.ShapeDtypeStruct((D, S), bf16),
        scratch_shapes=[
            pltpu.VMEM((G, S // 2, 128), u32),
            pltpu.VMEM((NQ, G, 64, TQ), u32),
            pltpu.VMEM((DP // 2, S), u32),
            pltpu.VMEM((DP // 2, TQ), u32),
            pltpu.VMEM((DIST, KC, 128), f32),
            pltpu.VMEM((NIT, HPI - 1, NE * VK, TQ), f32),
            pltpu.VMEM((HPI, (NOC - NE) * VK, TQ), f32),
            pltpu.VMEM((NQ, NIT, HPI * DH, TQ), f32),
            pltpu.VMEM((NIT, HPI, DH, NOC * VK, 128), f32),
            pltpu.VMEM((D, S), bf16),
            pltpu.VMEM((D, S), bf16),
            pltpu.VMEM((D, 3 * D), bf16),
            pltpu.VMEM((D, D), bf16),
            pltpu.VMEM((D, F), bf16),
            pltpu.VMEM((D, F), bf16),
            pltpu.VMEM((3 * D // 2, D), u32),
            pltpu.VMEM((D // 2, DP), u32),
            pltpu.VMEM((F // 2, DP), u32),
            pltpu.VMEM((D, 128), f32),
            pltpu.VMEM((128, 256), f32),
            pltpu.VMEM((F,), bf16),
            pltpu.VMEM((D,), bf16),
            pltpu.SemaphoreType.DMA((6,)),
            pltpu.SemaphoreType.DMA((1,)),
        ],
        compiler_params=pltpu.CompilerParams(
            dimension_semantics=("arbitrary",),
            vmem_limit_bytes=100 * 2**20,
            disable_bounds_checks=True,
        ),
        name="fused_block",
    )(A_x.reshape(S, D).T, A_wqkv, A_wo, B_w1, B_b1, B_w2.T, B_b2)
    return outT.T.reshape(1, S, D)
```

```python
import jax
import jax.numpy as jnp
from jax import lax
import jax.experimental.pallas as pl
import jax.experimental.pallas.tpu as pltpu

S, D, H, DH, F = 2048, 448, 16, 28, 1792
EPS = 1e-5
LOG2E = 1.4426950408889634
bf16, f32, u32 = jnp.bfloat16, jnp.float32, jnp.uint32

HP = 32
DP = H * HP
G = 4
GW = 4 * DH
TQ = 512
NQ = S // TQ
NT = TQ // 128
KC = 128
NKC = S // KC
HPI = 8
NIT = H // HPI
GPI = HPI // 4
DIST = 8

VK = 16
OCH = (4, 5, 6, 7, 9, 10, 11, 12, 13, 14, 15)
NE = 6
NOC = len(OCH)
_REST = [c for c in range(NKC) if c not in OCH]
CORD = _REST[:3] + list(OCH[NE:]) + list(OCH[:NE]) + _REST[3:]
EHEADS = [(hh, u) for hh in range(NIT) for u in range(1, HPI)]

XSPLIT = ((0, 256), (256, 512), (512, 1024), (1024, 1536), (1536, 2048))
WSPLIT = ((0, 512), (512, 896), (896, 1344))


def _pk(x):
    return pltpu.bitcast(x, u32)


def _up(x):
    return pltpu.bitcast(x, bf16)


def _dot(a, b):
    return jnp.dot(a, b, preferred_element_type=f32)


def _ln(x):
    m = jnp.sum(x, axis=0, keepdims=True) * (1.0 / D)
    xc = x - m
    v = jnp.sum(xc * xc, axis=0, keepdims=True) * (1.0 / D)
    return xc * lax.rsqrt(v + EPS)


def _pad_head_rows(w, fill):
    parts = []
    for h in range(H):
        parts += [w[DH * h:DH * (h + 1), :], fill]
    return jnp.concatenate(parts, axis=0)


def _first_row(row, rows):
    r = lax.broadcasted_iota(jnp.int32, (rows, row.shape[1]), 0)
    return jnp.where(r == 0, row, 0.0)


def _kernel(xT_hbm, wqkv_hbm, wo_hbm, w1_hbm, b1_hbm, w2T_hbm, b2_hbm,
            o_hbm,
            k_sc, qT_sc, vT_sc, oT_sc, spre_sc, sve_sc, sva_sc, qf_sc, kb_sc, y_sc,
            xT_ref, wqkv_ref, wo_ref, w1_ref, w2T_ref, w2p_sc, wqkvT_sc, woT_sc, w1T_sc, b2_sc, kt_sc,
            b1_ref, b2_ref, sems, osem):
    i = pl.program_id(0)
    rowq = lax.broadcasted_iota(jnp.int32, (64, TQ), 0)

    def masked_q(blk, g, j):
        qg = qT_sc[blk, g]
        keep = (rowq >= (DH // 2) * j) & (rowq < (DH // 2) * (j + 1))
        return _up(jnp.where(keep, qg, jnp.zeros_like(qg)))

    def qk(g, k0, k1, qm):
        return _dot(_up(k_sc[g, k0 // 2:k1 // 2, :]), qm)

    def vpu_scores(blk, hlist, o0, o1, rows):
        prev = jnp.zeros((rows, 128), f32)
        for hh, u in hlist:
            for t in range(NT):
                for v0 in range(o0 * VK, o1 * VK, rows):
                    a = prev * 0.0
                    for d in range(DH):
                        r = u * DH + d
                        a = a + kb_sc[hh, u, d, v0:v0 + rows, :] * qf_sc[blk, hh, r:r + 1, t * 128:(t + 1) * 128]
                    if o0 >= NE:
                        sva_sc[u, v0 - NE * VK:v0 - NE * VK + rows, t * 128:(t + 1) * 128] = a
                    else:
                        sve_sc[hh, u - 1, v0:v0 + rows, t * 128:(t + 1) * 128] = a
                    prev = a

    @pl.when(i == 0)
    def _prologue():
        def cp_x(n, sem):
            a, b = XSPLIT[n]
            return pltpu.make_async_copy(xT_hbm.at[:, a:b], xT_ref.at[:, a:b], sems.at[sem])

        def cp_w(n, sem):
            a, b = WSPLIT[n]
            return pltpu.make_async_copy(wqkv_hbm.at[:, a:b], wqkv_ref.at[:, a:b], sems.at[sem])

        def cp(src, dst, sem):
            return pltpu.make_async_copy(src, dst, sems.at[sem])

        stages = [
            [cp_x(0, 0)],
            [cp_w(0, 1)],
            [cp_x(1, 2), cp_w(1, 2)],
            [cp_w(2, 3), cp_x(2, 3)],
            [cp_x(3, 4), cp_x(4, 4), cp(wo_hbm, wo_ref, 4), cp(b2_hbm, b2_ref, 4), cp(b1_hbm, b1_ref, 4),
             cp(w1_hbm, w1_ref, 4)],
            [cp(w2T_hbm, w2T_ref, 5)],
        ]
        for st in stages:
            for c in st:
                c.start()

        def wait(n):
            for c in stages[n]:
                c.wait()

        def ln1(n):
            a, b = XSPLIT[n]
            return _ln(xT_ref[:, a:b].astype(f32)).astype(bf16)

        def transpose_w(n):
            a, b = WSPLIT[n]
            wqkvT_sc[a // 2:b // 2, :] = _pk(wqkv_ref[:, a:b].T)

        def proj(r0, r1, xn):
            return _dot(_up(wqkvT_sc[r0 // 2:r1 // 2, :]), xn)

        def proj_q(n, xn, g0=0, g1=G):
            a, b = XSPLIT[n]
            cols = slice(a % TQ, a % TQ + b - a)
            zpad = jnp.zeros((128 - GW, b - a), f32)
            qT = proj(GW * g0, GW * g1, xn) * (DH ** -0.5 * LOG2E)
            for g in range(g0, g1):
                qg = qT[GW * (g - g0):GW * (g - g0 + 1), :]
                qf_sc[a // TQ, g // GPI, GW * (g % GPI):GW * (g % GPI + 1), cols] = qg.astype(bf16).astype(f32)
                qT_sc[a // TQ, g, :, cols] = _pk(jnp.concatenate([qg, zpad], axis=0).astype(bf16))

        def proj_k(n, xn):
            a, b = XSPLIT[n]
            zpad = jnp.zeros((128 - GW, b - a), f32)
            kT = proj(D, 2 * D, xn)
            for g in range(G):
                kg = jnp.concatenate([kT[GW * g:GW * (g + 1), :], zpad], axis=0).astype(bf16)
                k_sc[g, a // 2:b // 2, :] = _pk(kg.T)

        def proj_v(n, xn):
            a, b = XSPLIT[n]
            ones = _first_row(jnp.ones((1, b - a), f32), HP - DH)
            vT_sc[:, a:b] = _pk(_pad_head_rows(proj(2 * D, 3 * D, xn), ones).astype(bf16))

        def vkeys(g, o0, o1):
            return jnp.concatenate(
                [k_sc[g, ((OCH[o] + 1) * KC - VK) // 2:(OCH[o] + 1) * KC // 2, :] for o in range(o0, o1)], axis=0)

        def broadcast_k(o0, o1, via_transpose):
            for j in range(4):
                sel = [(g, o0 if (4 * g + j) % HPI else max(o0, NE)) for g in range(G)]
                sel = [(g, lo) for g, lo in sel if lo < o1]
                ksel = jnp.concatenate([vkeys(g, lo, o1) for g, lo in sel], axis=0)
                nk = 2 * ksel.shape[0]
                if via_transpose:
                    kt_sc[:, 0:nk] = _up(ksel).T.astype(f32)
                for d in range(DH):
                    lane = DH * j + d
                    if via_transpose:
                        kb = jnp.broadcast_to(kt_sc[lane:lane + 1, 0:nk], (128, nk)).astype(bf16).T.astype(f32)
                    else:
                        kb = _up(jnp.broadcast_to(ksel[:, lane:lane + 1], ksel.shape)).astype(f32)
                    r0 = 0
                    for g, lo in sel:
                        h = 4 * g + j
                        kb_sc[h // HPI, h % HPI, d, lo * VK:o1 * VK, :] = kb[r0:r0 + (o1 - lo) * VK, :]
                        r0 += (o1 - lo) * VK

        def first_scores(hlist, o0, o1):
            for hh, u in hlist:
                h = hh * HPI + u
                s = _dot(_up(vkeys(h // 4, o0, o1)), masked_q(0, h // 4, h % 4))
                if o0 >= NE:
                    sva_sc[u, (o0 - NE) * VK:(o1 - NE) * VK, :] = s
                else:
                    sve_sc[hh, u - 1, o0 * VK:o1 * VK, :] = s

        wait(0)
        xn0 = ln1(0)
        wait(1)
        transpose_w(0)
        proj_q(0, xn0, 0, 3)
        wait(2)
        proj_q(0, xn0, 3, 4)
        transpose_w(1)
        xn1 = ln1(1)
        proj_k(0, xn0)
        proj_q(1, xn1)
        wait(3)
        proj_k(1, xn1)
        transpose_w(2)
        xn2 = ln1(2)
        proj_k(2, xn2)
        broadcast_k(0, 4, True)
        proj_v(0, xn0)
        proj_v(1, xn1)
        proj_q(2, xn2)
        proj_v(2, xn2)
        wait(4)
        woT_sc[...] = _pk(_pad_head_rows(wo_ref[...].astype(f32), jnp.zeros((HP - DH, D), f32)).astype(bf16).T)
        b2_sc[...] = jnp.broadcast_to(b2_ref[...].astype(f32).reshape(1, D), (128, D)).T
        b1_rows = _first_row(b1_ref[...].astype(f32).reshape(1, F), DP - D).astype(bf16)
        w1T_sc[...] = _pk(jnp.concatenate([w1_ref[...], b1_rows], axis=0).T)
        xn3 = ln1(3)
        first_scores(EHEADS, 0, 4)
        proj_k(3, xn3)
        xn4 = ln1(4)
        proj_k(4, xn4)
        broadcast_k(4, 7, False)
        broadcast_k(7, NOC, True)
        proj_v(3, xn3)
        proj_q(3, xn3)
        proj_v(4, xn4)
        proj_q(4, xn4)
        first_scores(EHEADS, 4, NE)
        first_scores([(0, u) for u in range(HPI)], NE, NOC)
        qm = masked_q(0, 0, 0)
        for w in range(DIST):
            c = CORD[w // NT]
            spre_sc[w] = qk(0, c * KC, (c + 1) * KC, qm[:, (w % NT) * 128:(w % NT + 1) * 128])
        wait(5)

    def attention(hh, carry):
        work = [(u, c, t) for u in range(HPI) for c in CORD for t in range(NT)]
        n = len(work)
        per_head = NKC * NT
        nxt = i * NIT + hh + 1
        nblk = jnp.minimum(nxt // NIT, NQ - 1)
        nhh = nxt % NIT
        qms = {}

        def scores(w):
            u, c, t = work[w % n]
            cols = slice(t * 128, (t + 1) * 128)
            if w >= n:
                if "next" not in qms:
                    qms["next"] = masked_q(nblk, nhh * GPI, 0)
                return qk(nhh * GPI, c * KC, (c + 1) * KC, qms["next"][:, cols])
            g = hh * GPI + u // 4
            if u not in qms:
                qms[u] = masked_q(i, g, u % 4)
            qm = qms[u][:, cols]
            if c in (OCH if u else OCH[NE:]):
                o = OCH.index(c)
                if o < NE:
                    sv = sve_sc[hh, u - 1, o * VK:(o + 1) * VK, cols]
                else:
                    sv = sva_sc[u, (o - NE) * VK:(o - NE + 1) * VK, cols]
                return jnp.concatenate([qk(g, c * KC, (c + 1) * KC - VK, qm), sv], axis=0)
            return qk(g, c * KC, (c + 1) * KC, qm)

        svals = {w: spre_sc[w] for w in range(DIST)}
        state = {}
        for w, (u, c, t) in enumerate(work):
            s = svals.pop(w)
            m, acc = state.get((u, t), (None, None))
            cm = jnp.max(s, axis=0, keepdims=True)
            m_new = cm if m is None else jnp.maximum(m, cm)
            p = jnp.exp2(s - m_new).astype(bf16)
            if w + DIST < n:
                svals[w + DIST] = scores(w + DIST)
            else:
                spre_sc[w + DIST - n] = scores(w + DIST)
            h0 = pl.multiple_of((hh * HPI + u) * (HP // 2), HP // 2)
            pv = _dot(_up(vT_sc[pl.ds(h0, HP // 2), c * KC:(c + 1) * KC]), p)
            acc = pv if m is None else acc * jnp.exp2(m - m_new) + pv
            state[(u, t)] = (m_new, acc)
            if w % per_head >= per_head - NT:
                l = acc[DH:DH + 1, :]
                r = pl.reciprocal(l, approx=True)
                r = r * (2.0 - l * r)
                oT_sc[pl.ds(h0, HP // 2), t * 128:(t + 1) * 128] = _pk((acc * r).astype(bf16))
        vpu_scores(nblk, [(nhh, u) for u in range(HPI)], NE, NOC, 8)
        return carry

    lax.fori_loop(0, NIT, attention, 0)

    q0 = pl.multiple_of(i * TQ, TQ)
    hT = xT_ref[:, pl.ds(q0, TQ)].astype(f32) + _dot(_up(woT_sc[...]), _up(oT_sc[...]))
    ones = _first_row(jnp.ones((1, 128), f32), DP - D)
    for t in range(NT):
        ht = hT[:, t * 128:(t + 1) * 128]
        hn = jnp.concatenate([_ln(ht), ones], axis=0).astype(bf16)
        u = jnp.maximum(_dot(_up(w1T_sc[...]), hn), 0.0)
        if t == 0:
            w2 = w2T_ref[...]
            w2p_sc[...] = _pk(w2)
        else:
            w2 = _up(w2p_sc[...])
        y = ht + b2_sc[...] + _dot(w2, (u * u).astype(bf16))
        y_sc[:, pl.ds(pl.multiple_of(q0 + t * 128, 128), 128)] = y.astype(bf16)
        if t >= NT - 2:
            c0, cw = (0, (NT - 1) * 128) if t == NT - 2 else (t * 128, 128)
            cols = pl.ds(pl.multiple_of(q0 + c0, 128), cw)
            pltpu.make_async_copy(y_sc.at[:, cols], o_hbm.at[:, cols], osem.at[0]).start()
    vpu_scores(jnp.minimum(i + 1, NQ - 1), EHEADS, 0, NE, 24)

    @pl.when(i == NQ - 1)
    def _():
        pltpu.make_async_copy(y_sc, o_hbm, osem.at[0]).wait()


@jax.jit
def pallas_sequential_preLN__mha_block__dense_activation_squared_relu__prompt_kernel(
    A_x: jax.Array,
    A_wqkv: jax.Array,
    A_wo: jax.Array,
    B_x: jax.Array,
    B_w1: jax.Array,
    B_b1: jax.Array,
    B_w2: jax.Array,
    B_b2: jax.Array,
):
    del B_x
    hbm = pl.BlockSpec(memory_space=pl.ANY)
    outT = pl.pallas_call(
        _kernel,
        grid=(NQ,),
        in_specs=[hbm] * 7,
        out_specs=hbm,
        out_shape=jax.ShapeDtypeStruct((D, S), bf16),
        scratch_shapes=[
            pltpu.VMEM((G, S // 2, 128), u32),
            pltpu.VMEM((NQ, G, 64, TQ), u32),
            pltpu.VMEM((DP // 2, S), u32),
            pltpu.VMEM((DP // 2, TQ), u32),
            pltpu.VMEM((DIST, KC, 128), f32),
            pltpu.VMEM((NIT, HPI - 1, NE * VK, TQ), f32),
            pltpu.VMEM((HPI, (NOC - NE) * VK, TQ), f32),
            pltpu.VMEM((NQ, NIT, HPI * DH, TQ), f32),
            pltpu.VMEM((NIT, HPI, DH, NOC * VK, 128), f32),
            pltpu.VMEM((D, S), bf16),
            pltpu.VMEM((D, S), bf16),
            pltpu.VMEM((D, 3 * D), bf16),
            pltpu.VMEM((D, D), bf16),
            pltpu.VMEM((D, F), bf16),
            pltpu.VMEM((D, F), bf16),
            pltpu.VMEM((D // 2, F), u32),
            pltpu.VMEM((3 * D // 2, D), u32),
            pltpu.VMEM((D // 2, DP), u32),
            pltpu.VMEM((F // 2, DP), u32),
            pltpu.VMEM((D, 128), f32),
            pltpu.VMEM((128, 256), f32),
            pltpu.VMEM((F,), bf16),
            pltpu.VMEM((D,), bf16),
            pltpu.SemaphoreType.DMA((6,)),
            pltpu.SemaphoreType.DMA((1,)),
        ],
        compiler_params=pltpu.CompilerParams(
            dimension_semantics=("arbitrary",),
            vmem_limit_bytes=100 * 2**20,
            disable_bounds_checks=True,
        ),
        name="fused_block",
    )(A_x.reshape(S, D).T, A_wqkv, A_wo, B_w1, B_b1, B_w2.T, B_b2)
    return outT.T.reshape(1, S, D)
```

```python
import jax
import jax.numpy as jnp
from jax import lax
import jax.experimental.pallas as pl
import jax.experimental.pallas.tpu as pltpu

S, D, H, DH, F = 2048, 448, 16, 28, 1792
EPS = 1e-5
LOG2E = 1.4426950408889634
bf16, f32, u32 = jnp.bfloat16, jnp.float32, jnp.uint32

HP = 32
DP = H * HP
G = 4
GW = 4 * DH
TQ = 512
NQ = S // TQ
NT = TQ // 128
KC = 128
NKC = S // KC
HPI = 8
NIT = H // HPI
GPI = HPI // 4
DIST = 8

VK = 16
OCH = (4, 5, 6, 7, 9, 10, 11, 12, 13, 14, 15)
NE = 6
NOC = len(OCH)
_REST = [c for c in range(NKC) if c not in OCH]
CORD = _REST[:3] + list(OCH[NE:]) + list(OCH[:NE]) + _REST[3:]
EHEADS = [(hh, u) for hh in range(NIT) for u in range(1, HPI)]

XSPLIT = ((0, 256), (256, 512), (512, 1024), (1024, 1536), (1536, 2048))
WSPLIT = ((0, 512), (512, 896), (896, 1344))


def _pk(x):
    return pltpu.bitcast(x, u32)


def _up(x):
    return pltpu.bitcast(x, bf16)


def _dot(a, b):
    return jnp.dot(a, b, preferred_element_type=f32)


def _ln(x):
    m = jnp.sum(x, axis=0, keepdims=True) * (1.0 / D)
    xc = x - m
    v = jnp.sum(xc * xc, axis=0, keepdims=True) * (1.0 / D)
    return xc * lax.rsqrt(v + EPS)


def _pad_head_rows(w, fill):
    parts = []
    for h in range(H):
        parts += [w[DH * h:DH * (h + 1), :], fill]
    return jnp.concatenate(parts, axis=0)


def _first_row(row, rows):
    r = lax.broadcasted_iota(jnp.int32, (rows, row.shape[1]), 0)
    return jnp.where(r == 0, row, 0.0)


def _kernel(xT_hbm, wqkv_hbm, wo_hbm, w1_hbm, b1_hbm, w2T_hbm, b2_hbm,
            o_hbm,
            k_sc, qT_sc, vT_sc, oT_sc, spre_sc, sve_sc, sva_sc, qf_sc, kb_sc, y_sc,
            xT_ref, wqkv_ref, wo_ref, w1_ref, w2T_ref, w2p_sc, wqkvT_sc, woT_sc, w1T_sc, b2_sc, kt_sc,
            b1_ref, b2_ref, sems, osem):
    i = pl.program_id(0)
    rowq = lax.broadcasted_iota(jnp.int32, (64, TQ), 0)

    def masked_q(blk, g, j):
        qg = qT_sc[blk, g]
        keep = (rowq >= (DH // 2) * j) & (rowq < (DH // 2) * (j + 1))
        return _up(jnp.where(keep, qg, jnp.zeros_like(qg)))

    def qk(g, k0, k1, qm):
        return _dot(_up(k_sc[g, k0 // 2:k1 // 2, :]), qm)

    def vpu_scores(blk, hlist, o0, o1, rows):
        prev = jnp.zeros((rows, 128), f32)
        for hh, u in hlist:
            for t in range(NT):
                for v0 in range(o0 * VK, o1 * VK, rows):
                    a = prev * 0.0
                    for d in range(DH):
                        r = u * DH + d
                        a = a + kb_sc[hh, u, d, v0:v0 + rows, :] * qf_sc[blk, hh, r:r + 1, t * 128:(t + 1) * 128]
                    if o0 >= NE:
                        sva_sc[u, v0 - NE * VK:v0 - NE * VK + rows, t * 128:(t + 1) * 128] = a
                    else:
                        sve_sc[hh, u - 1, v0:v0 + rows, t * 128:(t + 1) * 128] = a
                    prev = a

    @pl.when(i == 0)
    def _prologue():
        def cp_x(n, sem):
            a, b = XSPLIT[n]
            return pltpu.make_async_copy(xT_hbm.at[:, a:b], xT_ref.at[:, a:b], sems.at[sem])

        def cp_w(n, sem):
            a, b = WSPLIT[n]
            return pltpu.make_async_copy(wqkv_hbm.at[:, a:b], wqkv_ref.at[:, a:b], sems.at[sem])

        def cp(src, dst, sem):
            return pltpu.make_async_copy(src, dst, sems.at[sem])

        stages = [
            [cp_x(0, 0)],
            [cp_w(0, 1)],
            [cp_x(1, 2), cp_w(1, 2)],
            [cp_w(2, 3), cp_x(2, 3)],
            [cp_x(3, 4), cp_x(4, 4), cp(wo_hbm, wo_ref, 4), cp(b2_hbm, b2_ref, 4), cp(b1_hbm, b1_ref, 4),
             cp(w1_hbm, w1_ref, 4)],
            [cp(w2T_hbm, w2T_ref, 5)],
        ]
        for st in stages:
            for c in st:
                c.start()

        def wait(n):
            for c in stages[n]:
                c.wait()

        def ln1(n):
            a, b = XSPLIT[n]
            return _ln(xT_ref[:, a:b].astype(f32)).astype(bf16)

        def transpose_w(n):
            a, b = WSPLIT[n]
            wqkvT_sc[a // 2:b // 2, :] = _pk(wqkv_ref[:, a:b].T)

        def proj(r0, r1, xn):
            return _dot(_up(wqkvT_sc[r0 // 2:r1 // 2, :]), xn)

        def proj_q(n, xn, g0=0, g1=G):
            a, b = XSPLIT[n]
            cols = slice(a % TQ, a % TQ + b - a)
            zpad = jnp.zeros((128 - GW, b - a), f32)
            qT = proj(GW * g0, GW * g1, xn) * (DH ** -0.5 * LOG2E)
            for g in range(g0, g1):
                qg = qT[GW * (g - g0):GW * (g - g0 + 1), :]
                qf_sc[a // TQ, g // GPI, GW * (g % GPI):GW * (g % GPI + 1), cols] = qg.astype(bf16).astype(f32)
                qT_sc[a // TQ, g, :, cols] = _pk(jnp.concatenate([qg, zpad], axis=0).astype(bf16))

        def proj_k(n, xn):
            a, b = XSPLIT[n]
            zpad = jnp.zeros((128 - GW, b - a), f32)
            kT = proj(D, 2 * D, xn)
            for g in range(G):
                kg = jnp.concatenate([kT[GW * g:GW * (g + 1), :], zpad], axis=0).astype(bf16)
                k_sc[g, a // 2:b // 2, :] = _pk(kg.T)

        def proj_v(n, xn):
            a, b = XSPLIT[n]
            ones = _first_row(jnp.ones((1, b - a), f32), HP - DH)
            vT_sc[:, a:b] = _pk(_pad_head_rows(proj(2 * D, 3 * D, xn), ones).astype(bf16))

        def vkeys(g, o0, o1):
            return jnp.concatenate(
                [k_sc[g, ((OCH[o] + 1) * KC - VK) // 2:(OCH[o] + 1) * KC // 2, :] for o in range(o0, o1)], axis=0)

        def broadcast_k(o0, o1, via_transpose):
            for j in range(4):
                sel = [(g, o0 if (4 * g + j) % HPI else max(o0, NE)) for g in range(G)]
                sel = [(g, lo) for g, lo in sel if lo < o1]
                ksel = jnp.concatenate([vkeys(g, lo, o1) for g, lo in sel], axis=0)
                nk = 2 * ksel.shape[0]
                if via_transpose:
                    kt_sc[:, 0:nk] = _up(ksel).T.astype(f32)
                for d in range(DH):
                    lane = DH * j + d
                    if via_transpose:
                        kb = jnp.broadcast_to(kt_sc[lane:lane + 1, 0:nk], (128, nk)).astype(bf16).T.astype(f32)
                    else:
                        kb = _up(jnp.broadcast_to(ksel[:, lane:lane + 1], ksel.shape)).astype(f32)
                    r0 = 0
                    for g, lo in sel:
                        h = 4 * g + j
                        kb_sc[h // HPI, h % HPI, d, lo * VK:o1 * VK, :] = kb[r0:r0 + (o1 - lo) * VK, :]
                        r0 += (o1 - lo) * VK

        def first_scores(hlist, o0, o1):
            for hh, u in hlist:
                h = hh * HPI + u
                s = _dot(_up(vkeys(h // 4, o0, o1)), masked_q(0, h // 4, h % 4))
                if o0 >= NE:
                    sva_sc[u, (o0 - NE) * VK:(o1 - NE) * VK, :] = s
                else:
                    sve_sc[hh, u - 1, o0 * VK:o1 * VK, :] = s

        wait(0)
        xn0 = ln1(0)
        wait(1)
        transpose_w(0)
        proj_q(0, xn0, 0, 3)
        wait(2)
        proj_q(0, xn0, 3, 4)
        transpose_w(1)
        xn1 = ln1(1)
        proj_k(0, xn0)
        proj_q(1, xn1)
        wait(3)
        proj_k(1, xn1)
        transpose_w(2)
        xn2 = ln1(2)
        proj_k(2, xn2)
        broadcast_k(0, 4, True)
        proj_v(0, xn0)
        proj_v(1, xn1)
        proj_q(2, xn2)
        proj_v(2, xn2)
        wait(4)
        woT_sc[...] = _pk(_pad_head_rows(wo_ref[...].astype(f32), jnp.zeros((HP - DH, D), f32)).astype(bf16).T)
        b2_sc[...] = jnp.broadcast_to(b2_ref[...].astype(f32).reshape(1, D), (128, D)).T
        b1_rows = _first_row(b1_ref[...].astype(f32).reshape(1, F), DP - D).astype(bf16)
        w1T_sc[...] = _pk(jnp.concatenate([w1_ref[...], b1_rows], axis=0).T)
        xn3 = ln1(3)
        first_scores(EHEADS, 0, 4)
        proj_k(3, xn3)
        xn4 = ln1(4)
        proj_k(4, xn4)
        broadcast_k(4, 7, False)
        broadcast_k(7, NOC, True)
        proj_v(3, xn3)
        proj_q(3, xn3)
        proj_v(4, xn4)
        proj_q(4, xn4)
        first_scores(EHEADS, 4, NE)
        first_scores([(0, u) for u in range(HPI)], NE, NOC)
        qm = masked_q(0, 0, 0)
        for w in range(DIST):
            c = CORD[w // NT]
            spre_sc[w] = qk(0, c * KC, (c + 1) * KC, qm[:, (w % NT) * 128:(w % NT + 1) * 128])
        wait(5)

    def attention(hh, carry):
        work = [(u, c, t) for u in range(HPI) for c in CORD for t in range(NT)]
        n = len(work)
        per_head = NKC * NT
        nxt = i * NIT + hh + 1
        nblk = jnp.minimum(nxt // NIT, NQ - 1)
        nhh = nxt % NIT
        qms = {}

        def scores(w):
            u, c, t = work[w % n]
            cols = slice(t * 128, (t + 1) * 128)
            if w >= n:
                if "next" not in qms:
                    qms["next"] = masked_q(nblk, nhh * GPI, 0)
                return jnp.concatenate([qk(nhh * GPI, k0, k0 + KC // 4, qms["next"][:, cols])
                                        for k0 in range(c * KC, (c + 1) * KC, KC // 4)], axis=0)
            g = hh * GPI + u // 4
            if u not in qms:
                qms[u] = masked_q(i, g, u % 4)
            qm = qms[u][:, cols]
            if c in (OCH if u else OCH[NE:]):
                o = OCH.index(c)
                if o < NE:
                    sv = sve_sc[hh, u - 1, o * VK:(o + 1) * VK, cols]
                else:
                    sv = sva_sc[u, (o - NE) * VK:(o - NE + 1) * VK, cols]
                return jnp.concatenate([qk(g, c * KC, (c + 1) * KC - VK, qm), sv], axis=0)
            return qk(g, c * KC, (c + 1) * KC, qm)

        svals = {w: spre_sc[w] for w in range(DIST)}
        state = {}
        for w, (u, c, t) in enumerate(work):
            s = svals.pop(w)
            m, acc = state.get((u, t), (None, None))
            cm = jnp.max(s, axis=0, keepdims=True)
            m_new = cm if m is None else jnp.maximum(m, cm)
            p = jnp.exp2(s - m_new).astype(bf16)
            if w + DIST < n:
                svals[w + DIST] = scores(w + DIST)
            elif w < n - 2:
                spre_sc[w + DIST - n] = scores(w + DIST)
            h0 = pl.multiple_of((hh * HPI + u) * (HP // 2), HP // 2)
            pv = _dot(_up(vT_sc[pl.ds(h0, HP // 2), c * KC:(c + 1) * KC]), p)
            acc = pv if m is None else acc * jnp.exp2(m - m_new) + pv
            state[(u, t)] = (m_new, acc)
            if w % per_head >= per_head - NT:
                l = acc[DH:DH + 1, :]
                r = pl.reciprocal(l, approx=True)
                r = r * (2.0 - l * r)
                oT_sc[pl.ds(h0, HP // 2), t * 128:(t + 1) * 128] = _pk((acc * r).astype(bf16))
        for w in range(n - 2, n):
            spre_sc[w + DIST - n] = scores(w + DIST)
        vpu_scores(nblk, [(nhh, u) for u in range(HPI)], NE, NOC, 8)
        return carry

    lax.fori_loop(0, NIT, attention, 0)

    q0 = pl.multiple_of(i * TQ, TQ)
    hT = xT_ref[:, pl.ds(q0, TQ)].astype(f32) + _dot(_up(woT_sc[...]), _up(oT_sc[...]))
    ones = _first_row(jnp.ones((1, 128), f32), DP - D)
    for t in range(NT):
        ht = hT[:, t * 128:(t + 1) * 128]
        hn = jnp.concatenate([_ln(ht), ones], axis=0).astype(bf16)
        u = jnp.maximum(_dot(_up(w1T_sc[...]), hn), 0.0)
        if t == 0:
            w2 = w2T_ref[...]
            w2p_sc[...] = _pk(w2)
        else:
            w2 = _up(w2p_sc[...])
        y = ht + b2_sc[...] + _dot(w2, (u * u).astype(bf16))
        y_sc[:, pl.ds(pl.multiple_of(q0 + t * 128, 128), 128)] = y.astype(bf16)
        if t >= NT - 2:
            c0, cw = (0, (NT - 1) * 128) if t == NT - 2 else (t * 128, 128)
            cols = pl.ds(pl.multiple_of(q0 + c0, 128), cw)
            pltpu.make_async_copy(y_sc.at[:, cols], o_hbm.at[:, cols], osem.at[0]).start()
    vpu_scores(jnp.minimum(i + 1, NQ - 1), EHEADS, 0, NE, 24)

    @pl.when(i == NQ - 1)
    def _():
        pltpu.make_async_copy(y_sc, o_hbm, osem.at[0]).wait()


@jax.jit
def pallas_sequential_preLN__mha_block__dense_activation_squared_relu__prompt_kernel(
    A_x: jax.Array,
    A_wqkv: jax.Array,
    A_wo: jax.Array,
    B_x: jax.Array,
    B_w1: jax.Array,
    B_b1: jax.Array,
    B_w2: jax.Array,
    B_b2: jax.Array,
):
    del B_x
    hbm = pl.BlockSpec(memory_space=pl.ANY)
    outT = pl.pallas_call(
        _kernel,
        grid=(NQ,),
        in_specs=[hbm] * 7,
        out_specs=hbm,
        out_shape=jax.ShapeDtypeStruct((D, S), bf16),
        scratch_shapes=[
            pltpu.VMEM((G, S // 2, 128), u32),
            pltpu.VMEM((NQ, G, 64, TQ), u32),
            pltpu.VMEM((DP // 2, S), u32),
            pltpu.VMEM((DP // 2, TQ), u32),
            pltpu.VMEM((DIST, KC, 128), f32),
            pltpu.VMEM((NIT, HPI - 1, NE * VK, TQ), f32),
            pltpu.VMEM((HPI, (NOC - NE) * VK, TQ), f32),
            pltpu.VMEM((NQ, NIT, HPI * DH, TQ), f32),
            pltpu.VMEM((NIT, HPI, DH, NOC * VK, 128), f32),
            pltpu.VMEM((D, S), bf16),
            pltpu.VMEM((D, S), bf16),
            pltpu.VMEM((D, 3 * D), bf16),
            pltpu.VMEM((D, D), bf16),
            pltpu.VMEM((D, F), bf16),
            pltpu.VMEM((D, F), bf16),
            pltpu.VMEM((D // 2, F), u32),
            pltpu.VMEM((3 * D // 2, D), u32),
            pltpu.VMEM((D // 2, DP), u32),
            pltpu.VMEM((F // 2, DP), u32),
            pltpu.VMEM((D, 128), f32),
            pltpu.VMEM((128, 256), f32),
            pltpu.VMEM((F,), bf16),
            pltpu.VMEM((D,), bf16),
            pltpu.SemaphoreType.DMA((6,)),
            pltpu.SemaphoreType.DMA((1,)),
        ],
        compiler_params=pltpu.CompilerParams(
            dimension_semantics=("arbitrary",),
            vmem_limit_bytes=100 * 2**20,
            disable_bounds_checks=True,
        ),
        name="fused_block",
    )(A_x.reshape(S, D).T, A_wqkv, A_wo, B_w1, B_b1, B_w2.T, B_b2)
    return outT.T.reshape(1, S, D)
```

```python
import jax
import jax.numpy as jnp
from jax import lax
import jax.experimental.pallas as pl
import jax.experimental.pallas.tpu as pltpu

S, D, H, DH, F = 2048, 448, 16, 28, 1792
EPS = 1e-5
LOG2E = 1.4426950408889634
bf16, f32, u32 = jnp.bfloat16, jnp.float32, jnp.uint32

HP = 32
DP = H * HP
G = 4
GW = 4 * DH
TQ = 512
NQ = S // TQ
NT = TQ // 128
KC = 128
NKC = S // KC
HPI = 8
NIT = H // HPI
GPI = HPI // 4
DIST = 8

VK = 16
OCH = (4, 5, 2, 3, 6, 7, 13, 11, 12, 14, 15)
NE = 6
NOC = len(OCH)
_REST = [c for c in range(NKC) if c not in OCH]
CORD = _REST[:3] + list(OCH[NE:]) + list(OCH[:NE]) + _REST[3:]
EHEADS = [(hh, u) for hh in range(NIT) for u in range(1, HPI)]

XSPLIT = ((0, 256), (256, 512), (512, 1024), (1024, 1536), (1536, 2048))
WSPLIT = ((0, 512), (512, 896), (896, 1344))


def _pk(x):
    return pltpu.bitcast(x, u32)


def _up(x):
    return pltpu.bitcast(x, bf16)


def _dot(a, b):
    return jnp.dot(a, b, preferred_element_type=f32)


def _ln(x):
    m = jnp.sum(x, axis=0, keepdims=True) * (1.0 / D)
    xc = x - m
    v = jnp.sum(xc * xc, axis=0, keepdims=True) * (1.0 / D)
    return xc * lax.rsqrt(v + EPS)


def _pad_head_rows(w, fill):
    parts = []
    for h in range(H):
        parts += [w[DH * h:DH * (h + 1), :], fill]
    return jnp.concatenate(parts, axis=0)


def _first_row(row, rows):
    r = lax.broadcasted_iota(jnp.int32, (rows, row.shape[1]), 0)
    return jnp.where(r == 0, row, 0.0)


def _kernel(xT_hbm, wqkv_hbm, wo_hbm, w1_hbm, b1_hbm, w2T_hbm, b2_hbm,
            o_hbm,
            k_sc, qT_sc, vT_sc, oT_sc, spre_sc, sve_sc, sva_sc, qf_sc, kb_sc, y_sc,
            xT_ref, wqkv_ref, wo_ref, w1_ref, w2T_ref, w2p_sc, wqkvT_sc, woT_sc, w1T_sc, b2_sc, kt_sc,
            b1_ref, b2_ref, sems, osem):
    i = pl.program_id(0)
    rowq = lax.broadcasted_iota(jnp.int32, (64, TQ), 0)

    def masked_q(blk, g, j):
        qg = qT_sc[blk, g]
        keep = (rowq >= (DH // 2) * j) & (rowq < (DH // 2) * (j + 1))
        return _up(jnp.where(keep, qg, jnp.zeros_like(qg)))

    def qk(g, k0, k1, qm):
        return _dot(_up(k_sc[g, k0 // 2:k1 // 2, :]), qm)

    def vpu_scores(blk, hlist, o0, o1, rows):
        prev = jnp.zeros((rows, 128), f32)
        for hh, u in hlist:
            for t in range(NT):
                for v0 in range(o0 * VK, o1 * VK, rows):
                    a = prev * 0.0
                    for d in range(DH):
                        r = u * DH + d
                        a = a + kb_sc[hh, u, d, v0:v0 + rows, :] * qf_sc[blk, hh, r:r + 1, t * 128:(t + 1) * 128]
                    if o0 >= NE:
                        sva_sc[u, v0 - NE * VK:v0 - NE * VK + rows, t * 128:(t + 1) * 128] = a
                    else:
                        sve_sc[hh, u - 1, v0:v0 + rows, t * 128:(t + 1) * 128] = a
                    prev = a

    @pl.when(i == 0)
    def _prologue():
        def cp_x(n, sem):
            a, b = XSPLIT[n]
            return pltpu.make_async_copy(xT_hbm.at[:, a:b], xT_ref.at[:, a:b], sems.at[sem])

        def cp_w(n, sem):
            a, b = WSPLIT[n]
            return pltpu.make_async_copy(wqkv_hbm.at[:, a:b], wqkv_ref.at[:, a:b], sems.at[sem])

        def cp(src, dst, sem):
            return pltpu.make_async_copy(src, dst, sems.at[sem])

        stages = [
            [cp_x(0, 0)],
            [cp_w(0, 1)],
            [cp_x(1, 2), cp_w(1, 2)],
            [cp_w(2, 3), cp_x(2, 3)],
            [cp_x(3, 4), cp_x(4, 4), cp(wo_hbm, wo_ref, 4), cp(b2_hbm, b2_ref, 4), cp(b1_hbm, b1_ref, 4),
             cp(w1_hbm, w1_ref, 4)],
            [cp(w2T_hbm, w2T_ref, 5)],
        ]
        for st in stages:
            for c in st:
                c.start()

        def wait(n):
            for c in stages[n]:
                c.wait()

        def ln1(n):
            a, b = XSPLIT[n]
            return _ln(xT_ref[:, a:b].astype(f32)).astype(bf16)

        def transpose_w(n):
            a, b = WSPLIT[n]
            wqkvT_sc[a // 2:b // 2, :] = _pk(wqkv_ref[:, a:b].T)

        def proj(r0, r1, xn):
            return _dot(_up(wqkvT_sc[r0 // 2:r1 // 2, :]), xn)

        def proj_q(n, xn, g0=0, g1=G):
            a, b = XSPLIT[n]
            cols = slice(a % TQ, a % TQ + b - a)
            zpad = jnp.zeros((128 - GW, b - a), f32)
            qT = proj(GW * g0, GW * g1, xn) * (DH ** -0.5 * LOG2E)
            for g in range(g0, g1):
                qg = qT[GW * (g - g0):GW * (g - g0 + 1), :]
                qf_sc[a // TQ, g // GPI, GW * (g % GPI):GW * (g % GPI + 1), cols] = qg.astype(bf16).astype(f32)
                qT_sc[a // TQ, g, :, cols] = _pk(jnp.concatenate([qg, zpad], axis=0).astype(bf16))

        def proj_k(n, xn):
            a, b = XSPLIT[n]
            zpad = jnp.zeros((128 - GW, b - a), f32)
            kT = proj(D, 2 * D, xn)
            for g in range(G):
                kg = jnp.concatenate([kT[GW * g:GW * (g + 1), :], zpad], axis=0).astype(bf16)
                k_sc[g, a // 2:b // 2, :] = _pk(kg.T)

        def proj_v(n, xn):
            a, b = XSPLIT[n]
            ones = _first_row(jnp.ones((1, b - a), f32), HP - DH)
            vT_sc[:, a:b] = _pk(_pad_head_rows(proj(2 * D, 3 * D, xn), ones).astype(bf16))

        def vkeys(g, o0, o1):
            return jnp.concatenate(
                [k_sc[g, ((OCH[o] + 1) * KC - VK) // 2:(OCH[o] + 1) * KC // 2, :] for o in range(o0, o1)], axis=0)

        def broadcast_k(n, sets, js):
            nk = sum((hi - lo) * VK for _, lo, hi in sets)
            dup = max(128 // nk, 1)
            kt_sc[n, :, 0:nk * dup] = _up(jnp.concatenate([vkeys(*s) for s in sets * dup], axis=0)).T.astype(f32)
            part = lax.broadcasted_iota(jnp.int32, (1, nk * dup), 1) // nk
            for j in js:
                for d in range(0, DH, dup):
                    r = DH * j + d
                    row = kt_sc[n, r:r + 1, 0:nk * dup]
                    for e in range(1, dup):
                        row = jnp.where(part == e, kt_sc[n, r + e:r + e + 1, 0:nk * dup], row)
                    kb = jnp.broadcast_to(row, (128, nk * dup)).astype(bf16).T.astype(f32)
                    r0 = 0
                    for e in range(dup):
                        for g, lo, hi in sets:
                            h = 4 * g + j
                            kb_sc[h // HPI, h % HPI, d + e, lo * VK:hi * VK, :] = kb[r0:r0 + (hi - lo) * VK, :]
                            r0 += (hi - lo) * VK

        def first_scores(hlist, o0, o1):
            for hh, u in hlist:
                h = hh * HPI + u
                s = _dot(_up(vkeys(h // 4, o0, o1)), masked_q(0, h // 4, h % 4))
                if o0 >= NE:
                    sva_sc[u, (o0 - NE) * VK:(o1 - NE) * VK, :] = s
                else:
                    sve_sc[hh, u - 1, o0 * VK:o1 * VK, :] = s

        wait(0)
        xn0 = ln1(0)
        wait(1)
        transpose_w(0)
        proj_q(0, xn0, 0, 3)
        wait(2)
        proj_q(0, xn0, 3, 4)
        transpose_w(1)
        xn1 = ln1(1)
        proj_k(0, xn0)
        proj_q(1, xn1)
        wait(3)
        proj_k(1, xn1)
        transpose_w(2)
        xn2 = ln1(2)
        proj_k(2, xn2)
        broadcast_k(0, [(1, 0, 4), (3, 0, 4)], range(4))
        broadcast_k(1, [(0, 0, 4), (2, 0, 4)], range(1, 4))
        broadcast_k(2, [(0, 4, NE), (2, 4, NE)], range(1, 4))
        proj_v(0, xn0)
        proj_v(1, xn1)
        proj_q(2, xn2)
        proj_v(2, xn2)
        wait(4)
        woT_sc[...] = _pk(_pad_head_rows(wo_ref[...].astype(f32), jnp.zeros((HP - DH, D), f32)).astype(bf16).T)
        b2_sc[...] = jnp.broadcast_to(b2_ref[...].astype(f32).reshape(1, D), (128, D)).T
        b1_rows = _first_row(b1_ref[...].astype(f32).reshape(1, F), DP - D).astype(bf16)
        w1T_sc[...] = _pk(jnp.concatenate([w1_ref[...], b1_rows], axis=0).T)
        xn3 = ln1(3)
        first_scores(EHEADS, 0, 4)
        proj_k(3, xn3)
        xn4 = ln1(4)
        proj_k(4, xn4)
        broadcast_k(3, [(1, 4, 7), (3, 4, 7), (0, NE, 7), (2, NE, 7)], range(4))
        broadcast_k(4, [(g, 7, NOC) for g in range(G)], range(4))
        proj_v(3, xn3)
        proj_q(3, xn3)
        proj_q(4, xn4)
        proj_v(4, xn4)
        first_scores(EHEADS, 4, NE)
        first_scores([(0, u) for u in range(HPI)], NE, NOC)
        qm = masked_q(0, 0, 0)
        for w in range(DIST):
            c = CORD[w // NT]
            spre_sc[w] = qk(0, c * KC, (c + 1) * KC, qm[:, (w % NT) * 128:(w % NT + 1) * 128])
        wait(5)

    def attention(hh, carry):
        work = [(u, c, t) for u in range(HPI) for c in CORD for t in range(NT)]
        n = len(work)
        per_head = NKC * NT
        nxt = i * NIT + hh + 1
        nblk = jnp.minimum(nxt // NIT, NQ - 1)
        nhh = nxt % NIT
        qms = {}

        def scores(w):
            u, c, t = work[w % n]
            cols = slice(t * 128, (t + 1) * 128)
            if w >= n:
                if "next" not in qms:
                    qms["next"] = masked_q(nblk, nhh * GPI, 0)
                return jnp.concatenate([qk(nhh * GPI, k0, k0 + KC // 4, qms["next"][:, cols])
                                        for k0 in range(c * KC, (c + 1) * KC, KC // 4)], axis=0)
            g = hh * GPI + u // 4
            if u not in qms:
                qms[u] = masked_q(i, g, u % 4)
            qm = qms[u][:, cols]
            if c in (OCH if u else OCH[NE:]):
                o = OCH.index(c)
                if o < NE:
                    sv = sve_sc[hh, u - 1, o * VK:(o + 1) * VK, cols]
                else:
                    sv = sva_sc[u, (o - NE) * VK:(o - NE + 1) * VK, cols]
                return jnp.concatenate([qk(g, c * KC, (c + 1) * KC - VK, qm), sv], axis=0)
            return qk(g, c * KC, (c + 1) * KC, qm)

        svals = {w: spre_sc[w] for w in range(DIST)}
        state = {}
        for w, (u, c, t) in enumerate(work):
            s = svals.pop(w)
            m, acc = state.get((u, t), (None, None))
            cm = jnp.max(s, axis=0, keepdims=True)
            m_new = cm if m is None else jnp.maximum(m, cm)
            p = jnp.exp2(s - m_new).astype(bf16)
            if w + DIST < n:
                svals[w + DIST] = scores(w + DIST)
            elif w < n - 2:
                spre_sc[w + DIST - n] = scores(w + DIST)
            h0 = pl.multiple_of((hh * HPI + u) * (HP // 2), HP // 2)
            pv = _dot(_up(vT_sc[pl.ds(h0, HP // 2), c * KC:(c + 1) * KC]), p)
            acc = pv if m is None else acc * jnp.exp2(m - m_new) + pv
            state[(u, t)] = (m_new, acc)
            if w % per_head >= per_head - NT:
                l = acc[DH:DH + 1, :]
                r = pl.reciprocal(l, approx=True)
                r = r * (2.0 - l * r)
                oT_sc[pl.ds(h0, HP // 2), t * 128:(t + 1) * 128] = _pk((acc * r).astype(bf16))
        for w in range(n - 2, n):
            spre_sc[w + DIST - n] = scores(w + DIST)
        vpu_scores(nblk, [(nhh, u) for u in range(HPI)], NE, NOC, 8)
        return carry

    lax.fori_loop(0, NIT, attention, 0)

    q0 = pl.multiple_of(i * TQ, TQ)
    hT = xT_ref[:, pl.ds(q0, TQ)].astype(f32) + _dot(_up(woT_sc[...]), _up(oT_sc[...]))
    ones = _first_row(jnp.ones((1, 128), f32), DP - D)
    for t in range(NT):
        ht = hT[:, t * 128:(t + 1) * 128]
        hn = jnp.concatenate([_ln(ht), ones], axis=0).astype(bf16)
        u = jnp.maximum(_dot(_up(w1T_sc[...]), hn), 0.0)
        if t == 0:
            w2 = w2T_ref[...]
            w2p_sc[...] = _pk(w2)
        else:
            w2 = _up(w2p_sc[...])
        y = ht + b2_sc[...] + _dot(w2, (u * u).astype(bf16))
        y_sc[:, pl.ds(pl.multiple_of(q0 + t * 128, 128), 128)] = y.astype(bf16)
        if t >= NT - 2:
            c0, cw = (0, (NT - 1) * 128) if t == NT - 2 else (t * 128, 128)
            cols = pl.ds(pl.multiple_of(q0 + c0, 128), cw)
            pltpu.make_async_copy(y_sc.at[:, cols], o_hbm.at[:, cols], osem.at[0]).start()
    vpu_scores(jnp.minimum(i + 1, NQ - 1), EHEADS, 0, NE, 24)

    @pl.when(i == NQ - 1)
    def _():
        pltpu.make_async_copy(y_sc, o_hbm, osem.at[0]).wait()


@jax.jit
def pallas_sequential_preLN__mha_block__dense_activation_squared_relu__prompt_kernel(
    A_x: jax.Array,
    A_wqkv: jax.Array,
    A_wo: jax.Array,
    B_x: jax.Array,
    B_w1: jax.Array,
    B_b1: jax.Array,
    B_w2: jax.Array,
    B_b2: jax.Array,
):
    del B_x
    hbm = pl.BlockSpec(memory_space=pl.ANY)
    outT = pl.pallas_call(
        _kernel,
        grid=(NQ,),
        in_specs=[hbm] * 7,
        out_specs=hbm,
        out_shape=jax.ShapeDtypeStruct((D, S), bf16),
        scratch_shapes=[
            pltpu.VMEM((G, S // 2, 128), u32),
            pltpu.VMEM((NQ, G, 64, TQ), u32),
            pltpu.VMEM((DP // 2, S), u32),
            pltpu.VMEM((DP // 2, TQ), u32),
            pltpu.VMEM((DIST, KC, 128), f32),
            pltpu.VMEM((NIT, HPI - 1, NE * VK, TQ), f32),
            pltpu.VMEM((HPI, (NOC - NE) * VK, TQ), f32),
            pltpu.VMEM((NQ, NIT, HPI * DH, TQ), f32),
            pltpu.VMEM((NIT, HPI, DH, NOC * VK, 128), f32),
            pltpu.VMEM((D, S), bf16),
            pltpu.VMEM((D, S), bf16),
            pltpu.VMEM((D, 3 * D), bf16),
            pltpu.VMEM((D, D), bf16),
            pltpu.VMEM((D, F), bf16),
            pltpu.VMEM((D, F), bf16),
            pltpu.VMEM((D // 2, F), u32),
            pltpu.VMEM((3 * D // 2, D), u32),
            pltpu.VMEM((D // 2, DP), u32),
            pltpu.VMEM((F // 2, DP), u32),
            pltpu.VMEM((D, 128), f32),
            pltpu.VMEM((5, 128, 256), f32),
            pltpu.VMEM((F,), bf16),
            pltpu.VMEM((D,), bf16),
            pltpu.SemaphoreType.DMA((6,)),
            pltpu.SemaphoreType.DMA((1,)),
        ],
        compiler_params=pltpu.CompilerParams(
            dimension_semantics=("arbitrary",),
            vmem_limit_bytes=100 * 2**20,
            disable_bounds_checks=True,
        ),
        name="fused_block",
    )(A_x.reshape(S, D).T, A_wqkv, A_wo, B_w1, B_b1, B_w2.T, B_b2)
    return outT.T.reshape(1, S, D)
```

```python
import jax
import jax.numpy as jnp
from jax import lax
import jax.experimental.pallas as pl
import jax.experimental.pallas.tpu as pltpu

S, D, H, DH, F = 2048, 448, 16, 28, 1792
EPS = 1e-5
LOG2E = 1.4426950408889634
bf16, f32, u32 = jnp.bfloat16, jnp.float32, jnp.uint32

HP = 32
DP = H * HP
G = 4
GW = 4 * DH
TQ = 512
NQ = S // TQ
NT = TQ // 128
KC = 128
NKC = S // KC
HPI = 8
NIT = H // HPI
GPI = HPI // 4
DIST = 8

VK = 16
OCH = (4, 5, 2, 3, 6, 7, 13, 11, 12, 14, 15)
NE = 6
NOC = len(OCH)
_REST = [c for c in range(NKC) if c not in OCH]
CORD = _REST[:3] + list(OCH[NE:]) + list(OCH[:NE]) + _REST[3:]
EHEADS = [(hh, u) for hh in range(NIT) for u in range(1, HPI)]

XSPLIT = ((0, 256), (256, 512), (512, 1024), (1024, 1536), (1536, 2048))
WSPLIT = ((0, 128), (128, 512), (512, 896), (896, 1344))


def _pk(x):
    return pltpu.bitcast(x, u32)


def _up(x):
    return pltpu.bitcast(x, bf16)


def _dot(a, b):
    return jnp.dot(a, b, preferred_element_type=f32)


def _ln(x):
    m = jnp.sum(x, axis=0, keepdims=True) * (1.0 / D)
    xc = x - m
    v = jnp.sum(xc * xc, axis=0, keepdims=True) * (1.0 / D)
    return xc * lax.rsqrt(v + EPS)


def _pad_head_rows(w, fill):
    parts = []
    for h in range(H):
        parts += [w[DH * h:DH * (h + 1), :], fill]
    return jnp.concatenate(parts, axis=0)


def _first_row(row, rows):
    r = lax.broadcasted_iota(jnp.int32, (rows, row.shape[1]), 0)
    return jnp.where(r == 0, row, 0.0)


def _kernel(xT_hbm, wqkv_hbm, wo_hbm, w1_hbm, b1_hbm, w2T_hbm, b2_hbm,
            o_hbm,
            k_sc, qT_sc, vT_sc, oT_sc, spre_sc, sve_sc, sva_sc, qf_sc, kb_sc, y_sc,
            xT_ref, wqkv_ref, wo_ref, w1_ref, w2T_ref, w2p_sc, wqkvT_sc, woT_sc, w1T_sc, b2_sc, kt_sc,
            b1_ref, b2_ref, sems, osem):
    i = pl.program_id(0)
    rowq = lax.broadcasted_iota(jnp.int32, (64, TQ), 0)

    def masked_q(blk, g, j):
        qg = qT_sc[blk, g]
        keep = (rowq >= (DH // 2) * j) & (rowq < (DH // 2) * (j + 1))
        return _up(jnp.where(keep, qg, jnp.zeros_like(qg)))

    def qk(g, k0, k1, qm):
        return _dot(_up(k_sc[g, k0 // 2:k1 // 2, :]), qm)

    def vpu_scores(blk, hlist, o0, o1, rows):
        prev = jnp.zeros((rows, 128), f32)
        for hh, u in hlist:
            for t in range(NT):
                for v0 in range(o0 * VK, o1 * VK, rows):
                    a = prev * 0.0
                    for d in range(DH):
                        r = u * DH + d
                        a = a + kb_sc[hh, u, d, v0:v0 + rows, :] * qf_sc[blk, hh, r:r + 1, t * 128:(t + 1) * 128]
                    if o0 >= NE:
                        sva_sc[u, v0 - NE * VK:v0 - NE * VK + rows, t * 128:(t + 1) * 128] = a
                    else:
                        sve_sc[hh, u - 1, v0:v0 + rows, t * 128:(t + 1) * 128] = a
                    prev = a

    @pl.when(i == 0)
    def _prologue():
        def cp_x(n, sem):
            a, b = XSPLIT[n]
            return pltpu.make_async_copy(xT_hbm.at[:, a:b], xT_ref.at[:, a:b], sems.at[sem])

        def cp_w(n, sem):
            a, b = WSPLIT[n]
            return pltpu.make_async_copy(wqkv_hbm.at[:, a:b], wqkv_ref.at[:, a:b], sems.at[sem])

        def cp(src, dst, sem):
            return pltpu.make_async_copy(src, dst, sems.at[sem])

        stages = [
            [cp_x(0, 0), cp_w(0, 0)],
            [cp_w(1, 1)],
            [cp_x(1, 2), cp_w(2, 2)],
            [cp_w(3, 3), cp_x(2, 3)],
            [cp_x(3, 4), cp_x(4, 4), cp(wo_hbm, wo_ref, 4), cp(b2_hbm, b2_ref, 4), cp(b1_hbm, b1_ref, 4),
             cp(w1_hbm, w1_ref, 4)],
            [cp(w2T_hbm, w2T_ref, 5)],
        ]
        for st in stages:
            for c in st:
                c.start()

        def wait(n):
            for c in stages[n]:
                c.wait()

        def ln1(n):
            a, b = XSPLIT[n]
            return _ln(xT_ref[:, a:b].astype(f32)).astype(bf16)

        def transpose_w(n):
            a, b = WSPLIT[n]
            wqkvT_sc[a // 2:b // 2, :] = _pk(wqkv_ref[:, a:b].T)

        def proj(r0, r1, xn):
            return _dot(_up(wqkvT_sc[r0 // 2:r1 // 2, :]), xn)

        def proj_q(n, xn, g0=0, g1=G):
            a, b = XSPLIT[n]
            cols = slice(a % TQ, a % TQ + b - a)
            zpad = jnp.zeros((128 - GW, b - a), f32)
            qT = proj(GW * g0, GW * g1, xn) * (DH ** -0.5 * LOG2E)
            for g in range(g0, g1):
                qg = qT[GW * (g - g0):GW * (g - g0 + 1), :]
                qf_sc[a // TQ, g // GPI, GW * (g % GPI):GW * (g % GPI + 1), cols] = qg.astype(bf16).astype(f32)
                qT_sc[a // TQ, g, :, cols] = _pk(jnp.concatenate([qg, zpad], axis=0).astype(bf16))

        def proj_k(n, xn):
            a, b = XSPLIT[n]
            zpad = jnp.zeros((128 - GW, b - a), f32)
            kT = proj(D, 2 * D, xn)
            for g in range(G):
                kg = jnp.concatenate([kT[GW * g:GW * (g + 1), :], zpad], axis=0).astype(bf16)
                k_sc[g, a // 2:b // 2, :] = _pk(kg.T)

        def proj_v(n, xn):
            a, b = XSPLIT[n]
            ones = _first_row(jnp.ones((1, b - a), f32), HP - DH)
            vT_sc[:, a:b] = _pk(_pad_head_rows(proj(2 * D, 3 * D, xn), ones).astype(bf16))

        def vkeys(g, o0, o1):
            return jnp.concatenate(
                [k_sc[g, ((OCH[o] + 1) * KC - VK) // 2:(OCH[o] + 1) * KC // 2, :] for o in range(o0, o1)], axis=0)

        def broadcast_k(n, sets, js):
            nk = sum((hi - lo) * VK for _, lo, hi in sets)
            dup = max(128 // nk, 1)
            kt_sc[n, :, 0:nk * dup] = _up(jnp.concatenate([vkeys(*s) for s in sets * dup], axis=0)).T.astype(f32)
            part = lax.broadcasted_iota(jnp.int32, (1, nk * dup), 1) // nk
            for j in js:
                for d in range(0, DH, dup):
                    r = DH * j + d
                    row = kt_sc[n, r:r + 1, 0:nk * dup]
                    for e in range(1, dup):
                        row = jnp.where(part == e, kt_sc[n, r + e:r + e + 1, 0:nk * dup], row)
                    kb = jnp.broadcast_to(row, (128, nk * dup)).astype(bf16).T.astype(f32)
                    r0 = 0
                    for e in range(dup):
                        for g, lo, hi in sets:
                            h = 4 * g + j
                            kb_sc[h // HPI, h % HPI, d + e, lo * VK:hi * VK, :] = kb[r0:r0 + (hi - lo) * VK, :]
                            r0 += (hi - lo) * VK

        def first_scores(hlist, o0, o1):
            for hh, u in hlist:
                h = hh * HPI + u
                s = _dot(_up(vkeys(h // 4, o0, o1)), masked_q(0, h // 4, h % 4))
                if o0 >= NE:
                    sva_sc[u, (o0 - NE) * VK:(o1 - NE) * VK, :] = s
                else:
                    sve_sc[hh, u - 1, o0 * VK:o1 * VK, :] = s

        wait(0)
        xn0 = ln1(0)
        transpose_w(0)
        wait(1)
        proj_q(0, xn0, 0, 1)
        transpose_w(1)
        proj_q(0, xn0, 1, 3)
        wait(2)
        proj_q(0, xn0, 3, 4)
        transpose_w(2)
        xn1 = ln1(1)
        proj_k(0, xn0)
        proj_q(1, xn1)
        wait(3)
        proj_k(1, xn1)
        transpose_w(3)
        xn2 = ln1(2)
        proj_k(2, xn2)
        broadcast_k(0, [(1, 0, 4), (3, 0, 4)], range(4))
        broadcast_k(1, [(0, 0, 4), (2, 0, 4)], range(1, 4))
        broadcast_k(2, [(0, 4, NE), (2, 4, NE)], range(1, 4))
        proj_v(0, xn0)
        proj_v(1, xn1)
        proj_q(2, xn2)
        proj_v(2, xn2)
        wait(4)
        woT_sc[...] = _pk(_pad_head_rows(wo_ref[...].astype(f32), jnp.zeros((HP - DH, D), f32)).astype(bf16).T)
        b2_sc[...] = jnp.broadcast_to(b2_ref[...].astype(f32).reshape(1, D), (128, D)).T
        b1_rows = _first_row(b1_ref[...].astype(f32).reshape(1, F), DP - D).astype(bf16)
        w1T_sc[...] = _pk(jnp.concatenate([w1_ref[...], b1_rows], axis=0).T)
        xn3 = ln1(3)
        first_scores(EHEADS, 0, 4)
        proj_k(3, xn3)
        xn4 = ln1(4)
        proj_k(4, xn4)
        broadcast_k(3, [(1, 4, 7), (3, 4, 7), (0, NE, 7), (2, NE, 7)], range(4))
        broadcast_k(4, [(g, 7, NOC) for g in range(G)], range(4))
        proj_v(3, xn3)
        proj_q(3, xn3)
        proj_q(4, xn4)
        proj_v(4, xn4)
        first_scores(EHEADS, 4, NE)
        first_scores([(0, u) for u in range(HPI)], NE, NOC)
        qm = masked_q(0, 0, 0)
        for w in range(DIST):
            c = CORD[w // NT]
            spre_sc[w] = qk(0, c * KC, (c + 1) * KC, qm[:, (w % NT) * 128:(w % NT + 1) * 128])
        wait(5)

    def attention(hh, carry):
        work = [(u, c, t) for u in range(HPI) for c in CORD for t in range(NT)]
        n = len(work)
        per_head = NKC * NT
        nxt = i * NIT + hh + 1
        nblk = jnp.minimum(nxt // NIT, NQ - 1)
        nhh = nxt % NIT
        qms = {}

        def scores(w):
            u, c, t = work[w % n]
            cols = slice(t * 128, (t + 1) * 128)
            if w >= n:
                if "next" not in qms:
                    qms["next"] = masked_q(nblk, nhh * GPI, 0)
                return jnp.concatenate([qk(nhh * GPI, k0, k0 + KC // 4, qms["next"][:, cols])
                                        for k0 in range(c * KC, (c + 1) * KC, KC // 4)], axis=0)
            g = hh * GPI + u // 4
            if u not in qms:
                qms[u] = masked_q(i, g, u % 4)
            qm = qms[u][:, cols]
            if c in (OCH if u else OCH[NE:]):
                o = OCH.index(c)
                if o < NE:
                    sv = sve_sc[hh, u - 1, o * VK:(o + 1) * VK, cols]
                else:
                    sv = sva_sc[u, (o - NE) * VK:(o - NE + 1) * VK, cols]
                return jnp.concatenate([qk(g, c * KC, (c + 1) * KC - VK, qm), sv], axis=0)
            return qk(g, c * KC, (c + 1) * KC, qm)

        svals = {w: spre_sc[w] for w in range(DIST)}
        state = {}
        for w, (u, c, t) in enumerate(work):
            s = svals.pop(w)
            m, acc = state.get((u, t), (None, None))
            cm = jnp.max(s, axis=0, keepdims=True)
            m_new = cm if m is None else jnp.maximum(m, cm)
            p = jnp.exp2(s - m_new).astype(bf16)
            if w + DIST < n:
                svals[w + DIST] = scores(w + DIST)
            elif w < n - 2:
                spre_sc[w + DIST - n] = scores(w + DIST)
            h0 = pl.multiple_of((hh * HPI + u) * (HP // 2), HP // 2)
            pv = _dot(_up(vT_sc[pl.ds(h0, HP // 2), c * KC:(c + 1) * KC]), p)
            acc = pv if m is None else acc * jnp.exp2(m - m_new) + pv
            state[(u, t)] = (m_new, acc)
            if w % per_head >= per_head - NT:
                l = acc[DH:DH + 1, :]
                r = pl.reciprocal(l, approx=True)
                r = r * (2.0 - l * r)
                oT_sc[pl.ds(h0, HP // 2), t * 128:(t + 1) * 128] = _pk((acc * r).astype(bf16))
        for w in range(n - 2, n):
            spre_sc[w + DIST - n] = scores(w + DIST)
        vpu_scores(nblk, [(nhh, u) for u in range(HPI)], NE, NOC, 8)
        return carry

    lax.fori_loop(0, NIT, attention, 0)

    q0 = pl.multiple_of(i * TQ, TQ)
    hT = xT_ref[:, pl.ds(q0, TQ)].astype(f32) + _dot(_up(woT_sc[...]), _up(oT_sc[...]))
    ones = _first_row(jnp.ones((1, 128), f32), DP - D)
    for t in range(NT):
        ht = hT[:, t * 128:(t + 1) * 128]
        hn = jnp.concatenate([_ln(ht), ones], axis=0).astype(bf16)
        u = jnp.maximum(_dot(_up(w1T_sc[...]), hn), 0.0)
        if t == 0:
            w2 = w2T_ref[...]
            w2p_sc[...] = _pk(w2)
        else:
            w2 = _up(w2p_sc[...])
        y = ht + b2_sc[...] + _dot(w2, (u * u).astype(bf16))
        y_sc[:, pl.ds(pl.multiple_of(q0 + t * 128, 128), 128)] = y.astype(bf16)
        if t >= NT - 2:
            c0, cw = (0, (NT - 1) * 128) if t == NT - 2 else (t * 128, 128)
            cols = pl.ds(pl.multiple_of(q0 + c0, 128), cw)
            pltpu.make_async_copy(y_sc.at[:, cols], o_hbm.at[:, cols], osem.at[0]).start()
    vpu_scores(jnp.minimum(i + 1, NQ - 1), EHEADS, 0, NE, 24)

    @pl.when(i == NQ - 1)
    def _():
        pltpu.make_async_copy(y_sc, o_hbm, osem.at[0]).wait()


@jax.jit
def pallas_sequential_preLN__mha_block__dense_activation_squared_relu__prompt_kernel(
    A_x: jax.Array,
    A_wqkv: jax.Array,
    A_wo: jax.Array,
    B_x: jax.Array,
    B_w1: jax.Array,
    B_b1: jax.Array,
    B_w2: jax.Array,
    B_b2: jax.Array,
):
    del B_x
    hbm = pl.BlockSpec(memory_space=pl.ANY)
    outT = pl.pallas_call(
        _kernel,
        grid=(NQ,),
        in_specs=[hbm] * 7,
        out_specs=hbm,
        out_shape=jax.ShapeDtypeStruct((D, S), bf16),
        scratch_shapes=[
            pltpu.VMEM((G, S // 2, 128), u32),
            pltpu.VMEM((NQ, G, 64, TQ), u32),
            pltpu.VMEM((DP // 2, S), u32),
            pltpu.VMEM((DP // 2, TQ), u32),
            pltpu.VMEM((DIST, KC, 128), f32),
            pltpu.VMEM((NIT, HPI - 1, NE * VK, TQ), f32),
            pltpu.VMEM((HPI, (NOC - NE) * VK, TQ), f32),
            pltpu.VMEM((NQ, NIT, HPI * DH, TQ), f32),
            pltpu.VMEM((NIT, HPI, DH, NOC * VK, 128), f32),
            pltpu.VMEM((D, S), bf16),
            pltpu.VMEM((D, S), bf16),
            pltpu.VMEM((D, 3 * D), bf16),
            pltpu.VMEM((D, D), bf16),
            pltpu.VMEM((D, F), bf16),
            pltpu.VMEM((D, F), bf16),
            pltpu.VMEM((D // 2, F), u32),
            pltpu.VMEM((3 * D // 2, D), u32),
            pltpu.VMEM((D // 2, DP), u32),
            pltpu.VMEM((F // 2, DP), u32),
            pltpu.VMEM((D, 128), f32),
            pltpu.VMEM((5, 128, 256), f32),
            pltpu.VMEM((F,), bf16),
            pltpu.VMEM((D,), bf16),
            pltpu.SemaphoreType.DMA((6,)),
            pltpu.SemaphoreType.DMA((1,)),
        ],
        compiler_params=pltpu.CompilerParams(
            dimension_semantics=("arbitrary",),
            vmem_limit_bytes=100 * 2**20,
            disable_bounds_checks=True,
        ),
        name="fused_block",
    )(A_x.reshape(S, D).T, A_wqkv, A_wo, B_w1, B_b1, B_w2.T, B_b2)
    return outT.T.reshape(1, S, D)
```
